```python
import os as _os
_os.environ.setdefault('JAX_PLATFORMS', 'cpu')
import jax
import jax.numpy as jnp

def _softmax(x, axis=-1):
    return jax.nn.softmax(x, axis=axis)

def _gelu(x):
    return jax.nn.gelu(x, approximate=True)

def _silu(x):
    return jax.nn.silu(x)

def _sigmoid(x):
    return jax.nn.sigmoid(x)

def _layernorm(x, axis=-1, eps=1e-05):
    m = jnp.mean(x, axis=axis, keepdims=True)
    v = jnp.var(x, axis=axis, keepdims=True)
    return (x - m) / jnp.sqrt(v + eps)

def _scatter_add(tgt, idx, src, axis=0):
    return tgt.at[idx].add(src)

def _segment_sum(src, seg, n):
    return jax.ops.segment_sum(src, seg, n)

class _Rng:

    def __init__(self, key):
        self._k = key

    def _next(self):
        self._k, sub = jax.random.split(self._k)
        return sub

    def normal(self, shape):
        return jax.random.normal(self._next(), shape, dtype=jnp.bfloat16)

    def randint(self, lo, hi, shape):
        return jax.random.randint(self._next(), shape, lo, hi, dtype=jnp.int32)

    def uniform(self, shape, lo=0.0, hi=1.0):
        return jax.random.uniform(self._next(), shape, jnp.bfloat16, lo, hi)

    def permutation(self, n):
        return jax.random.permutation(self._next(), n)
kernel_name = 'parallel_sum__memory_aug_recurrent_mem_tr__dense_activation_silu__prompt'

def setup_inputs():
    _rng = _Rng(jax.random.key(int.from_bytes(__import__("os").urandom(4), "little")))
    _w = lambda a: (lambda t: t.astype(jnp.bfloat16) if jnp.issubdtype(t.dtype, jnp.floating) else t)(jnp.asarray(a))

    def _A_setup():
        B, S, Dm = (1, 2048, 448)
        H, Dh = (16, 256)
        M, seg = (8, 32)
        seg = min(seg, S)
        S = S // seg * seg
        return {'x': _w((lambda *s: _rng.normal(s) * 0.05)(B, S, Dm)), 'mem0': _w((lambda *s: _rng.normal(s) * 0.2)(B, M, Dm)), 'Wq': _w((lambda *s: _rng.normal(s) * 0.8)(Dm, H, Dh) * Dm ** (-0.5)), 'Wk': _w((lambda *s: _rng.normal(s) * 0.8)(Dm, H, Dh) * Dm ** (-0.5)), 'Wv': _w((lambda *s: _rng.normal(s) * 0.2)(Dm, H, Dh) * Dm ** (-0.5)), 'Wo': _w((lambda *s: _rng.normal(s) * 0.2)(H, Dh, Dm) * (H * Dh) ** (-0.5)), 'seg_len': seg}
    _A_in = _A_setup()

    def _B_setup():
        B, S, D, F = (1, 2048, 448, 1792)
        return {'x': _w((lambda *s: _rng.normal(s) * 0.05)(B, S, D)), 'w1': _w((lambda *s: _rng.normal(s) * 0.05)(D, F) * D ** (-0.5)), 'w2': _w((lambda *s: _rng.normal(s) * 0.05)(F, D) * F ** (-0.5))}
    _B_in = _B_setup()
    return {'A_x': _A_in['x'], 'A_mem0': _A_in['mem0'], 'A_Wq': _A_in['Wq'], 'A_Wk': _A_in['Wk'], 'A_Wv': _A_in['Wv'], 'A_Wo': _A_in['Wo'], 'A_seg_len': _A_in['seg_len'], 'B_x': _B_in['x'], 'B_w1': _B_in['w1'], 'B_w2': _B_in['w2']}

def reference(A_x, A_mem0, A_Wq, A_Wk, A_Wv, A_Wo, A_seg_len, B_x, B_w1, B_w2):

    def _A_ref(x, mem0, Wq, Wk, Wv, Wo, seg_len):
        B, S, Dm = x.shape
        H, Dh = (Wq.shape[1], Wq.shape[2])
        M = mem0.shape[1]
        scale = Dh ** (-0.5)
        n_seg = S // seg_len
        L = M + seg_len
        idx = jnp.arange(L)
        mask = (idx[:, None] < M) | (idx[:, None] >= idx[None, :])
        mem = mem0
        outs = []
        for s in range(n_seg):
            xs = x[:, s * seg_len:(s + 1) * seg_len, :].copy()
            h = jnp.concatenate([mem, xs], axis=1)
            q = jnp.einsum('btd,dhe->bhte', h, Wq)
            k = jnp.einsum('btd,dhe->bhte', h, Wk)
            v = jnp.einsum('btd,dhe->bhte', h, Wv)
            scores = jnp.einsum('bhqe,bhke->bhqk', q, k) * scale
            scores = jnp.where(mask[None, None], scores, -1000000000.0)
            p = _softmax(scores, axis=-1)
            o = jnp.einsum('bhqk,bhke->bhqe', p, v)
            o = jnp.einsum('bhte,hed->btd', o, Wo)
            mem = o[:, :M, :].copy()
            outs.append(o[:, M:, :])
        return jnp.concatenate(outs, axis=1)

    def _B_ref(x, w1, w2):
        h = jnp.einsum('bsd,df->bsf', x, w1)
        h = _silu(h)
        out = jnp.einsum('bsf,fd->bsd', h, w2)
        return out
    x = A_x
    xn = _layernorm(x, axis=-1)
    return x + _A_ref(xn, A_mem0, A_Wq, A_Wk, A_Wv, A_Wo, A_seg_len) + _B_ref(xn, B_w1, B_w2)
```

```python
import functools

import jax
import jax.numpy as jnp
import jax.experimental.pallas as pl
import jax.experimental.pallas.tpu as pltpu

_LN_EPS = 1e-05
_NEG = -1000000000.0


def _kernel(x_ref, mem0_ref, wq_ref, wk_ref, wv_ref, wo_ref, w1_ref, w2_ref,
            o_ref, h_scr, o_scr, *, M, SEG, H, DH):
    s = pl.program_id(0)
    L = M + SEG
    scale = DH ** (-0.5)

    @pl.when(s == 0)
    def _():
        h_scr[0:M, :] = mem0_ref[0].astype(jnp.float32)

    x = x_ref[0].astype(jnp.float32)
    mu = jnp.mean(x, axis=-1, keepdims=True)
    xc = x - mu
    var = jnp.mean(xc * xc, axis=-1, keepdims=True)
    xn = xc / jnp.sqrt(var + _LN_EPS)
    h_scr[M:L, :] = xn
    xn_bf = xn.astype(jnp.bfloat16)

    h = h_scr[...].astype(jnp.bfloat16)
    q = jnp.dot(h, wq_ref[...], preferred_element_type=jnp.float32).astype(jnp.bfloat16)
    k = jnp.dot(h, wk_ref[...], preferred_element_type=jnp.float32).astype(jnp.bfloat16)
    v = jnp.dot(h, wv_ref[...], preferred_element_type=jnp.float32).astype(jnp.bfloat16)

    row = jax.lax.broadcasted_iota(jnp.int32, (L, L), 0)
    col = jax.lax.broadcasted_iota(jnp.int32, (L, L), 1)
    mask = (row < M) | (row >= col)

    for hd in range(H):
        sl = slice(hd * DH, (hd + 1) * DH)
        sc = jax.lax.dot_general(q[:, sl], k[:, sl], (((1,), (1,)), ((), ())),
                                 preferred_element_type=jnp.float32) * scale
        sc = jnp.where(mask, sc, _NEG)
        mx = jnp.max(sc, axis=-1, keepdims=True)
        e = jnp.exp(sc - mx)
        p = e / jnp.sum(e, axis=-1, keepdims=True)
        o_scr[:, sl] = jnp.dot(p.astype(jnp.bfloat16), v[:, sl],
                               preferred_element_type=jnp.float32)

    att = jnp.dot(o_scr[...].astype(jnp.bfloat16), wo_ref[...],
                  preferred_element_type=jnp.float32)

    h1 = jnp.dot(xn_bf, w1_ref[...], preferred_element_type=jnp.float32)
    h1 = h1 * jax.nn.sigmoid(h1)
    ffn = jnp.dot(h1.astype(jnp.bfloat16), w2_ref[...],
                  preferred_element_type=jnp.float32)

    o_ref[0] = (x + att[M:L, :] + ffn).astype(o_ref.dtype)
    h_scr[0:M, :] = att[0:M, :]


@functools.partial(jax.jit, static_argnames=("A_seg_len",))
def pallas_parallel_sum__memory_aug_recurrent_mem_tr__dense_activation_silu__prompt_kernel(
    A_x: jax.Array,
    A_mem0: jax.Array,
    A_Wq: jax.Array,
    A_Wk: jax.Array,
    A_Wv: jax.Array,
    A_Wo: jax.Array,
    A_seg_len,
    B_x: jax.Array,
    B_w1: jax.Array,
    B_w2: jax.Array,
):
    B, S, D = A_x.shape
    H, DH = A_Wq.shape[1], A_Wq.shape[2]
    M = A_mem0.shape[1]
    SEG = int(A_seg_len)
    F = B_w1.shape[1]
    n_seg = S // SEG
    L = M + SEG

    wq = A_Wq.reshape(D, H * DH)
    wk = A_Wk.reshape(D, H * DH)
    wv = A_Wv.reshape(D, H * DH)
    wo = A_Wo.reshape(H * DH, D)

    const2 = lambda s: (0, 0)
    kernel = functools.partial(_kernel, M=M, SEG=SEG, H=H, DH=DH)
    return pl.pallas_call(
        kernel,
        grid=(n_seg,),
        in_specs=[
            pl.BlockSpec((1, SEG, D), lambda s: (0, s, 0)),
            pl.BlockSpec((1, M, D), lambda s: (0, 0, 0)),
            pl.BlockSpec((D, H * DH), const2),
            pl.BlockSpec((D, H * DH), const2),
            pl.BlockSpec((D, H * DH), const2),
            pl.BlockSpec((H * DH, D), const2),
            pl.BlockSpec((D, F), const2),
            pl.BlockSpec((F, D), const2),
        ],
        out_specs=pl.BlockSpec((1, SEG, D), lambda s: (0, s, 0)),
        out_shape=jax.ShapeDtypeStruct((B, S, D), A_x.dtype),
        scratch_shapes=[
            pltpu.VMEM((L, D), jnp.float32),
            pltpu.VMEM((L, H * DH), jnp.float32),
        ],
        compiler_params=pltpu.CompilerParams(
            dimension_semantics=("arbitrary",),
            vmem_limit_bytes=100 * 1024 * 1024,
        ),
    )(A_x, A_mem0, wq, wk, wv, wo, B_w1, B_w2)
```

```python
import functools, os
import jax, jax.numpy as jnp
import jax.experimental.pallas as pl
import jax.experimental.pallas.tpu as pltpu
_LN_EPS = 1e-05
_NEG = -1000000000.0
_LOG2E = 1.4426950408889634
NT = (((1,), (1,)), ((), ()))

def _kernel(x_ref, mem0_ref, wq_ref, wk_ref, wv_ref, wo_ref, w1_ref, w2_ref,
            o_ref, xn_scr, xb_scr, lo_scr, h_scr, qkv_scr, o_scr, s_scr, m_scr, *, M, SEG, H, DH, N_SEG):
    s = pl.program_id(0)
    L = M + SEG
    RA = SEG - M
    HD = H * DH
    scale = DH ** (-0.5)
    CH = 128
    SPC = CH // SEG

    @pl.when(s == 0)
    def _():
        h_scr[0:M, :] = mem0_ref[0].astype(jnp.float32)
        row = jax.lax.broadcasted_iota(jnp.int32, (L, L), 0)
        col = jax.lax.broadcasted_iota(jnp.int32, (L, L), 1)
        mk = ((row < M) | (row >= col)).astype(jnp.float32)
        for hd in range(H):
            m_scr[hd * L:(hd + 1) * L, :] = mk

        def ln_chunk(c, carry):
            r0 = pl.multiple_of(c * CH, CH)
            x = x_ref[0, pl.ds(r0, CH), :].astype(jnp.float32)
            mu = jnp.mean(x, axis=-1, keepdims=True)
            xc = x - mu
            var = jnp.mean(xc * xc, axis=-1, keepdims=True)
            xn = xc / jnp.sqrt(var + _LN_EPS)
            xn_scr[pl.ds(r0, CH), :] = xn
            for j in range(SPC):
                b0 = pl.multiple_of((c * SPC + j) * M, M)
                xb_scr[pl.ds(b0, M), :] = xn[j * SEG + RA:(j + 1) * SEG, :]
            return carry
        jax.lax.fori_loop(0, (N_SEG * SEG) // CH, ln_chunk, 0)

        def lo_chunk(c, carry):
            r0 = pl.multiple_of(c * CH, CH)
            lhs = xb_scr[pl.ds(r0, CH), :].astype(jnp.bfloat16)
            lo_scr[pl.ds(r0, CH), 0:HD] = jnp.dot(lhs, wq_ref[...], preferred_element_type=jnp.float32)
            lo_scr[pl.ds(r0, CH), HD:2 * HD] = jnp.dot(lhs, wk_ref[...], preferred_element_type=jnp.float32)
            lo_scr[pl.ds(r0, CH), 2 * HD:3 * HD] = jnp.dot(lhs, wv_ref[...], preferred_element_type=jnp.float32)
            return carry
        jax.lax.fori_loop(0, (N_SEG * M) // CH, lo_chunk, 0)

    r0 = pl.multiple_of(s * SEG, SEG)
    x = x_ref[0, pl.ds(r0, SEG), :].astype(jnp.float32)
    xn = xn_scr[pl.ds(r0, SEG), :]
    xn_bf = xn.astype(jnp.bfloat16)
    h_scr[M:M + RA, :] = xn[0:RA, :]
    lhs = h_scr[...].astype(jnp.bfloat16)
    qkv_scr[0:M + RA, 0:HD] = jnp.dot(lhs, wq_ref[...], preferred_element_type=jnp.float32)
    qkv_scr[0:M + RA, HD:2 * HD] = jnp.dot(lhs, wk_ref[...], preferred_element_type=jnp.float32)
    qkv_scr[0:M + RA, 2 * HD:3 * HD] = jnp.dot(lhs, wv_ref[...], preferred_element_type=jnp.float32)
    b0 = pl.multiple_of(s * M, M)
    qkv_scr[M + RA:L, :] = lo_scr[pl.ds(b0, M), :]

    for hd in range(H):
        q = qkv_scr[:, hd * DH:(hd + 1) * DH].astype(jnp.bfloat16)
        k = qkv_scr[:, HD + hd * DH:HD + (hd + 1) * DH].astype(jnp.bfloat16)
        s_scr[hd * L:(hd + 1) * L, :] = jax.lax.dot_general(q, k, NT, preferred_element_type=jnp.float32)
    sc = jnp.where(m_scr[...] > 0, s_scr[...], _NEG)
    mx = jnp.max(sc, axis=-1, keepdims=True)
    e = jnp.exp2((sc - mx) * (scale * _LOG2E))
    den = jnp.sum(e, axis=-1, keepdims=True)
    r = pl.reciprocal(den, approx=True)
    r = r * (2.0 - den * r)
    r = r * (2.0 - den * r)
    s_scr[...] = e * r
    for hd in range(H):
        v = qkv_scr[:, 2 * HD + hd * DH:2 * HD + (hd + 1) * DH].astype(jnp.bfloat16)
        p = s_scr[hd * L:(hd + 1) * L, :].astype(jnp.bfloat16)
        o_scr[:, hd * DH:(hd + 1) * DH] = jnp.dot(p, v, preferred_element_type=jnp.float32)
    att = jnp.dot(o_scr[...].astype(jnp.bfloat16), wo_ref[...], preferred_element_type=jnp.float32)
    h1 = jnp.dot(xn_bf, w1_ref[...], preferred_element_type=jnp.float32)
    h1 = h1 * jax.nn.sigmoid(h1)
    ffn = jnp.dot(h1.astype(jnp.bfloat16), w2_ref[...], preferred_element_type=jnp.float32)
    o_ref[0] = (x + att[M:L, :] + ffn).astype(o_ref.dtype)
    h_scr[0:M, :] = att[0:M, :]

@functools.partial(jax.jit, static_argnames=("A_seg_len",))
def pallas_parallel_sum__memory_aug_recurrent_mem_tr__dense_activation_silu__prompt_kernel(
    A_x, A_mem0, A_Wq, A_Wk, A_Wv, A_Wo, A_seg_len, B_x, B_w1, B_w2):
    B, S, D = A_x.shape
    H, DH = A_Wq.shape[1], A_Wq.shape[2]
    M = A_mem0.shape[1]; SEG = int(A_seg_len); F = B_w1.shape[1]
    n_seg = S // SEG; L = M + SEG
    wq = A_Wq.reshape(D, H * DH); wk = A_Wk.reshape(D, H * DH); wv = A_Wv.reshape(D, H * DH)
    wo = A_Wo.reshape(H * DH, D)
    const2 = lambda s: (0, 0)
    one = pl.Buffered(1)
    kernel = functools.partial(_kernel, M=M, SEG=SEG, H=H, DH=DH, N_SEG=n_seg)
    return pl.pallas_call(kernel, grid=(n_seg,),
        in_specs=[pl.BlockSpec((1, S, D), lambda s: (0, 0, 0), pipeline_mode=one),
            pl.BlockSpec((1, M, D), lambda s: (0, 0, 0), pipeline_mode=one),
            pl.BlockSpec((D, H * DH), const2, pipeline_mode=one), pl.BlockSpec((D, H * DH), const2, pipeline_mode=one),
            pl.BlockSpec((D, H * DH), const2, pipeline_mode=one),
            pl.BlockSpec((H * DH, D), const2, pipeline_mode=one), pl.BlockSpec((D, F), const2, pipeline_mode=one),
            pl.BlockSpec((F, D), const2, pipeline_mode=one)],
        out_specs=pl.BlockSpec((1, SEG, D), lambda s: (0, s, 0)),
        out_shape=jax.ShapeDtypeStruct((B, S, D), A_x.dtype),
        scratch_shapes=[pltpu.VMEM((S, D), jnp.float32),
                        pltpu.VMEM((n_seg * M, D), jnp.float32),
                        pltpu.VMEM((n_seg * M, 3 * H * DH), jnp.float32),
                        pltpu.VMEM((SEG, D), jnp.float32),
                        pltpu.VMEM((L, 3 * H * DH), jnp.float32),
                        pltpu.VMEM((L, H * DH), jnp.float32),
                        pltpu.VMEM((H * L, L), jnp.float32),
                        pltpu.VMEM((H * L, L), jnp.float32)],
        compiler_params=pltpu.CompilerParams(dimension_semantics=("arbitrary",), vmem_limit_bytes=72 * 1024 * 1024),
    )(A_x, A_mem0, wq, wk, wv, wo, B_w1, B_w2)
```

```python
import functools, os
import jax, jax.numpy as jnp
import jax.experimental.pallas as pl
import jax.experimental.pallas.tpu as pltpu
_LN_EPS = 1e-05
_NEG = -1000000000.0
_LOG2E = 1.4426950408889634
NT = (((1,), (1,)), ((), ()))

def _kernel(x_ref, mem0_ref, wq_ref, wk_ref, wv_ref, wo_ref, w1_ref, w2_ref,
            o_ref, xn_scr, xb_scr, lo_scr, h_scr, qkv_scr, o_scr, s_scr, m_scr, *, M, SEG, H, DH, N_SEG):
    s = pl.program_id(0)
    L = M + SEG
    RA = SEG - M
    HD = H * DH
    scale = DH ** (-0.5)
    CH = 128
    SPC = CH // SEG

    @pl.when(s == 0)
    def _():
        h_scr[0:M, :] = mem0_ref[0].astype(jnp.float32)
        row = jax.lax.broadcasted_iota(jnp.int32, (L, L), 0)
        col = jax.lax.broadcasted_iota(jnp.int32, (L, L), 1)
        mk = ((row < M) | (row >= col)).astype(jnp.float32)
        for hd in range(H):
            m_scr[hd * L:(hd + 1) * L, :] = mk

        def ln_chunk(c, carry):
            r0 = pl.multiple_of(c * CH, CH)
            x = x_ref[0, pl.ds(r0, CH), :].astype(jnp.float32)
            mu = jnp.mean(x, axis=-1, keepdims=True)
            xc = x - mu
            var = jnp.mean(xc * xc, axis=-1, keepdims=True)
            xn = xc / jnp.sqrt(var + _LN_EPS)
            xn_scr[pl.ds(r0, CH), :] = xn
            for j in range(SPC):
                b0 = pl.multiple_of((c * SPC + j) * M, M)
                xb_scr[pl.ds(b0, M), :] = xn[j * SEG + RA:(j + 1) * SEG, :]
            return carry
        jax.lax.fori_loop(0, (N_SEG * SEG) // CH, ln_chunk, 0)

        def lo_chunk(c, carry):
            r0 = pl.multiple_of(c * CH, CH)
            lhs = xb_scr[pl.ds(r0, CH), :].astype(jnp.bfloat16)
            lo_scr[pl.ds(r0, CH), 0:HD] = jnp.dot(lhs, wq_ref[...], preferred_element_type=jnp.float32)
            lo_scr[pl.ds(r0, CH), HD:2 * HD] = jnp.dot(lhs, wk_ref[...], preferred_element_type=jnp.float32)
            lo_scr[pl.ds(r0, CH), 2 * HD:3 * HD] = jnp.dot(lhs, wv_ref[...], preferred_element_type=jnp.float32)
            return carry
        jax.lax.fori_loop(0, (N_SEG * M) // CH, lo_chunk, 0)

    r0 = pl.multiple_of(s * SEG, SEG)
    x = x_ref[0, pl.ds(r0, SEG), :].astype(jnp.float32)
    xn = xn_scr[pl.ds(r0, SEG), :]
    xn_bf = xn.astype(jnp.bfloat16)
    h_scr[M:M + RA, :] = xn[0:RA, :]
    lhs = h_scr[...].astype(jnp.bfloat16)
    b0 = pl.multiple_of(s * M, M)
    HG = H // 2
    KS = ((0, 256), (256, 448))
    GC = HG * DH

    def proj(w_ref, c0, dst):
        acc = None
        for k0, k1 in KS:
            part = jnp.dot(lhs[:, k0:k1], w_ref[k0:k1, c0:c0 + GC], preferred_element_type=jnp.float32)
            acc = part if acc is None else acc + part
        qkv_scr[0:M + RA, dst:dst + GC] = acc
        qkv_scr[M + RA:L, dst:dst + GC] = lo_scr[pl.ds(b0, M), dst:dst + GC]

    def scores(g):
        for hh in range(HG):
            hd = g * HG + hh
            q = qkv_scr[:, hd * DH:(hd + 1) * DH].astype(jnp.bfloat16)
            k = qkv_scr[:, HD + hd * DH:HD + (hd + 1) * DH].astype(jnp.bfloat16)
            s_scr[hd * L:(hd + 1) * L, :] = jax.lax.dot_general(q, k, NT, preferred_element_type=jnp.float32)

    def softmax(g):
        r0g, r1g = g * HG * L, (g + 1) * HG * L
        sc = jnp.where(m_scr[r0g:r1g, :] > 0, s_scr[r0g:r1g, :], _NEG)
        mx = jnp.max(sc, axis=-1, keepdims=True)
        e = jnp.exp2((sc - mx) * (scale * _LOG2E))
        den = jnp.sum(e, axis=-1, keepdims=True)
        r = pl.reciprocal(den, approx=True)
        r = r * (2.0 - den * r)
        r = r * (2.0 - den * r)
        s_scr[r0g:r1g, :] = e * r

    def pv(g):
        for hh in range(HG):
            hd = g * HG + hh
            v = qkv_scr[:, 2 * HD + hd * DH:2 * HD + (hd + 1) * DH].astype(jnp.bfloat16)
            p = s_scr[hd * L:(hd + 1) * L, :].astype(jnp.bfloat16)
            o_scr[:, hd * DH:(hd + 1) * DH] = jnp.dot(p, v, preferred_element_type=jnp.float32)

    def wo(g):
        return jnp.dot(o_scr[:, g * GC:(g + 1) * GC].astype(jnp.bfloat16), wo_ref[g * GC:(g + 1) * GC, :],
                       preferred_element_type=jnp.float32)

    proj(wq_ref, 0, 0); proj(wk_ref, 0, HD)
    scores(0)
    proj(wq_ref, GC, GC); proj(wk_ref, GC, HD + GC)
    softmax(0)
    scores(1)
    proj(wv_ref, 0, 2 * HD)
    softmax(1)
    pv(0)
    proj(wv_ref, GC, 2 * HD + GC)
    pv(1)
    att = wo(0) + wo(1)
    h1 = jnp.dot(xn_bf, w1_ref[...], preferred_element_type=jnp.float32)
    h1 = h1 * jax.nn.sigmoid(h1)
    ffn = jnp.dot(h1.astype(jnp.bfloat16), w2_ref[...], preferred_element_type=jnp.float32)
    o_ref[0] = (x + att[M:L, :] + ffn).astype(o_ref.dtype)
    h_scr[0:M, :] = att[0:M, :]

@functools.partial(jax.jit, static_argnames=("A_seg_len",))
def pallas_parallel_sum__memory_aug_recurrent_mem_tr__dense_activation_silu__prompt_kernel(
    A_x, A_mem0, A_Wq, A_Wk, A_Wv, A_Wo, A_seg_len, B_x, B_w1, B_w2):
    B, S, D = A_x.shape
    H, DH = A_Wq.shape[1], A_Wq.shape[2]
    M = A_mem0.shape[1]; SEG = int(A_seg_len); F = B_w1.shape[1]
    n_seg = S // SEG; L = M + SEG
    wq = A_Wq.reshape(D, H * DH); wk = A_Wk.reshape(D, H * DH); wv = A_Wv.reshape(D, H * DH)
    wo = A_Wo.reshape(H * DH, D)
    const2 = lambda s: (0, 0)
    one = pl.Buffered(1)
    kernel = functools.partial(_kernel, M=M, SEG=SEG, H=H, DH=DH, N_SEG=n_seg)
    return pl.pallas_call(kernel, grid=(n_seg,),
        in_specs=[pl.BlockSpec((1, S, D), lambda s: (0, 0, 0), pipeline_mode=one),
            pl.BlockSpec((1, M, D), lambda s: (0, 0, 0), pipeline_mode=one),
            pl.BlockSpec((D, H * DH), const2, pipeline_mode=one), pl.BlockSpec((D, H * DH), const2, pipeline_mode=one),
            pl.BlockSpec((D, H * DH), const2, pipeline_mode=one),
            pl.BlockSpec((H * DH, D), const2, pipeline_mode=one), pl.BlockSpec((D, F), const2, pipeline_mode=one),
            pl.BlockSpec((F, D), const2, pipeline_mode=one)],
        out_specs=pl.BlockSpec((1, SEG, D), lambda s: (0, s, 0)),
        out_shape=jax.ShapeDtypeStruct((B, S, D), A_x.dtype),
        scratch_shapes=[pltpu.VMEM((S, D), jnp.float32),
                        pltpu.VMEM((n_seg * M, D), jnp.float32),
                        pltpu.VMEM((n_seg * M, 3 * H * DH), jnp.float32),
                        pltpu.VMEM((SEG, D), jnp.float32),
                        pltpu.VMEM((L, 3 * H * DH), jnp.float32),
                        pltpu.VMEM((L, H * DH), jnp.float32),
                        pltpu.VMEM((H * L, L), jnp.float32),
                        pltpu.VMEM((H * L, L), jnp.float32)],
        compiler_params=pltpu.CompilerParams(dimension_semantics=("arbitrary",), vmem_limit_bytes=72 * 1024 * 1024),
    )(A_x, A_mem0, wq, wk, wv, wo, B_w1, B_w2)
```

```python
import functools, os
import jax, jax.numpy as jnp
import jax.experimental.pallas as pl
import jax.experimental.pallas.tpu as pltpu
_LN_EPS = 1e-05
_NEG = -1000000000.0
_LOG2E = 1.4426950408889634
NT = (((1,), (1,)), ((), ()))

def _kernel(x_ref, mem0_ref, wq_ref, wk_ref, wv_ref, wo_ref, w1_ref, w2_ref,
            o_ref, xn_scr, xb_scr, lo_scr, h_scr, qkv_scr, o_scr, s_scr, m_scr, olo_scr, part_scr, *, M, SEG, H, DH, N_SEG):
    s = pl.program_id(0)
    L = M + SEG
    RA = SEG - M
    HD = H * DH
    scale = DH ** (-0.5)
    CH = 128
    SPC = CH // SEG

    @pl.when(s == 0)
    def _():
        h_scr[0:M, :] = mem0_ref[0].astype(jnp.float32)
        row = jax.lax.broadcasted_iota(jnp.int32, (L, L), 0)
        col = jax.lax.broadcasted_iota(jnp.int32, (L, L), 1)
        mk = ((row < M) | (row >= col)).astype(jnp.float32)
        for hd in range(H):
            m_scr[hd * L:(hd + 1) * L, :] = mk

        def ln_chunk(c, carry):
            r0 = pl.multiple_of(c * CH, CH)
            x = x_ref[0, pl.ds(r0, CH), :].astype(jnp.float32)
            mu = jnp.mean(x, axis=-1, keepdims=True)
            xc = x - mu
            var = jnp.mean(xc * xc, axis=-1, keepdims=True)
            xn = xc / jnp.sqrt(var + _LN_EPS)
            xn_scr[pl.ds(r0, CH), :] = xn
            for j in range(SPC):
                b0 = pl.multiple_of((c * SPC + j) * M, M)
                xb_scr[pl.ds(b0, M), :] = xn[j * SEG + RA:(j + 1) * SEG, :]
            return carry
        jax.lax.fori_loop(0, (N_SEG * SEG) // CH, ln_chunk, 0)

        def lo_chunk(c, carry):
            r0 = pl.multiple_of(c * CH, CH)
            lhs = xb_scr[pl.ds(r0, CH), :].astype(jnp.bfloat16)
            lo_scr[pl.ds(r0, CH), 0:HD] = jnp.dot(lhs, wq_ref[...], preferred_element_type=jnp.float32)
            lo_scr[pl.ds(r0, CH), HD:2 * HD] = jnp.dot(lhs, wk_ref[...], preferred_element_type=jnp.float32)
            lo_scr[pl.ds(r0, CH), 2 * HD:3 * HD] = jnp.dot(lhs, wv_ref[...], preferred_element_type=jnp.float32)
            return carry
        jax.lax.fori_loop(0, (N_SEG * M) // CH, lo_chunk, 0)

    r0 = pl.multiple_of(s * SEG, SEG)
    x = x_ref[0, pl.ds(r0, SEG), :].astype(jnp.float32)
    xn = xn_scr[pl.ds(r0, SEG), :]
    xn_bf = xn.astype(jnp.bfloat16)
    h_scr[M:M + RA, :] = xn[0:RA, :]
    lhs = h_scr[...].astype(jnp.bfloat16)
    b0 = pl.multiple_of(s * M, M)
    HG = H // 2
    KS = ((0, 256), (256, 448))
    GC = HG * DH

    def proj(w_ref, c0, dst):
        acc = None
        for k0, k1 in KS:
            part = jnp.dot(lhs[:, k0:k1], w_ref[k0:k1, c0:c0 + GC], preferred_element_type=jnp.float32)
            acc = part if acc is None else acc + part
        qkv_scr[0:M + RA, dst:dst + GC] = acc
        qkv_scr[M + RA:L, dst:dst + GC] = lo_scr[pl.ds(b0, M), dst:dst + GC]

    def scores(g):
        for hh in range(HG):
            hd = g * HG + hh
            q = qkv_scr[:, hd * DH:(hd + 1) * DH].astype(jnp.bfloat16)
            k = qkv_scr[:, HD + hd * DH:HD + (hd + 1) * DH].astype(jnp.bfloat16)
            s_scr[hd * L:(hd + 1) * L, :] = jax.lax.dot_general(q, k, NT, preferred_element_type=jnp.float32)

    def softmax(g):
        r0g, r1g = g * HG * L, (g + 1) * HG * L
        sc = jnp.where(m_scr[r0g:r1g, :] > 0, s_scr[r0g:r1g, :] * scale, _NEG)
        mx = jnp.max(sc, axis=-1, keepdims=True)
        e = jnp.exp2((sc - mx) * _LOG2E)
        den = jnp.sum(e, axis=-1, keepdims=True)
        r = pl.reciprocal(den, approx=True)
        r = r * (2.0 - den * r)
        r = r * (2.0 - den * r)
        s_scr[r0g:r1g, :] = e * r

    def pv(g):
        for hh in range(HG):
            hd = g * HG + hh
            v = qkv_scr[:, 2 * HD + hd * DH:2 * HD + (hd + 1) * DH].astype(jnp.bfloat16)
            p = s_scr[hd * L:(hd + 1) * L, :].astype(jnp.bfloat16)
            o_scr[:, hd * DH:(hd + 1) * DH] = jnp.dot(p, v, preferred_element_type=jnp.float32)

    def wo(g):
        return jnp.dot(o_scr[0:M + RA, g * GC:(g + 1) * GC].astype(jnp.bfloat16), wo_ref[g * GC:(g + 1) * GC, :],
                       preferred_element_type=jnp.float32)

    proj(wq_ref, 0, 0); proj(wk_ref, 0, HD)
    scores(0)
    proj(wq_ref, GC, GC); proj(wk_ref, GC, HD + GC)
    softmax(0)
    scores(1)
    proj(wv_ref, 0, 2 * HD)
    softmax(1)
    pv(0)
    proj(wv_ref, GC, 2 * HD + GC)
    pv(1)
    att = wo(0) + wo(1)
    h1 = jnp.dot(xn_bf, w1_ref[...], preferred_element_type=jnp.float32)
    h1 = h1 * jax.nn.sigmoid(h1)
    ffn = jnp.dot(h1.astype(jnp.bfloat16), w2_ref[...], preferred_element_type=jnp.float32)
    o_ref[0, pl.ds(r0, RA), :] = (x[0:RA, :] + att[M:M + RA, :] + ffn[0:RA, :]).astype(o_ref.dtype)
    h_scr[0:M, :] = att[0:M, :]
    olo_scr[pl.ds(b0, M), :] = o_scr[M + RA:L, :]
    part_scr[pl.ds(b0, M), :] = x[RA:SEG, :] + ffn[RA:SEG, :]

    @pl.when(s == N_SEG - 1)
    def _():
        for c in range((N_SEG * M) // CH):
            a = jnp.dot(olo_scr[c * CH:(c + 1) * CH, :].astype(jnp.bfloat16), wo_ref[...],
                        preferred_element_type=jnp.float32) + part_scr[c * CH:(c + 1) * CH, :]
            for j in range(CH // M):
                seg = c * (CH // M) + j
                o_ref[0, seg * SEG + RA:(seg + 1) * SEG, :] = a[j * M:(j + 1) * M, :].astype(o_ref.dtype)

@functools.partial(jax.jit, static_argnames=("A_seg_len",))
def pallas_parallel_sum__memory_aug_recurrent_mem_tr__dense_activation_silu__prompt_kernel(
    A_x, A_mem0, A_Wq, A_Wk, A_Wv, A_Wo, A_seg_len, B_x, B_w1, B_w2):
    B, S, D = A_x.shape
    H, DH = A_Wq.shape[1], A_Wq.shape[2]
    M = A_mem0.shape[1]; SEG = int(A_seg_len); F = B_w1.shape[1]
    n_seg = S // SEG; L = M + SEG
    wq = A_Wq.reshape(D, H * DH); wk = A_Wk.reshape(D, H * DH); wv = A_Wv.reshape(D, H * DH)
    wo = A_Wo.reshape(H * DH, D)
    const2 = lambda s: (0, 0)
    one = pl.Buffered(1)
    kernel = functools.partial(_kernel, M=M, SEG=SEG, H=H, DH=DH, N_SEG=n_seg)
    return pl.pallas_call(kernel, grid=(n_seg,),
        in_specs=[pl.BlockSpec((1, S, D), lambda s: (0, 0, 0), pipeline_mode=one),
            pl.BlockSpec((1, M, D), lambda s: (0, 0, 0), pipeline_mode=one),
            pl.BlockSpec((D, H * DH), const2, pipeline_mode=one), pl.BlockSpec((D, H * DH), const2, pipeline_mode=one),
            pl.BlockSpec((D, H * DH), const2, pipeline_mode=one),
            pl.BlockSpec((H * DH, D), const2, pipeline_mode=one), pl.BlockSpec((D, F), const2, pipeline_mode=one),
            pl.BlockSpec((F, D), const2, pipeline_mode=one)],
        out_specs=pl.BlockSpec((1, S, D), lambda s: (0, 0, 0)),
        out_shape=jax.ShapeDtypeStruct((B, S, D), A_x.dtype),
        scratch_shapes=[pltpu.VMEM((S, D), jnp.float32),
                        pltpu.VMEM((n_seg * M, D), jnp.float32),
                        pltpu.VMEM((n_seg * M, 3 * H * DH), jnp.float32),
                        pltpu.VMEM((SEG, D), jnp.float32),
                        pltpu.VMEM((L, 3 * H * DH), jnp.float32),
                        pltpu.VMEM((L, H * DH), jnp.float32),
                        pltpu.VMEM((H * L, L), jnp.float32),
                        pltpu.VMEM((H * L, L), jnp.float32),
                        pltpu.VMEM((n_seg * M, H * DH), jnp.float32),
                        pltpu.VMEM((n_seg * M, D), jnp.float32)],
        compiler_params=pltpu.CompilerParams(dimension_semantics=("arbitrary",), vmem_limit_bytes=80 * 1024 * 1024),
    )(A_x, A_mem0, wq, wk, wv, wo, B_w1, B_w2)
```
